```python
import jax
import jax.numpy as jnp

def _softmax(x, axis=-1):
    return jax.nn.softmax(x, axis=axis)
def _gelu(x):
    return jax.nn.gelu(x, approximate=True)
def _silu(x):
    return jax.nn.silu(x)
def _sigmoid(x):
    return jax.nn.sigmoid(x)
def _layernorm(x, axis=-1, eps=1e-5):
    m = jnp.mean(x, axis=axis, keepdims=True)
    v = jnp.var(x, axis=axis, keepdims=True)
    return (x - m) / jnp.sqrt(v + eps)
def _scatter_add(tgt, idx, src, axis=0):
    return tgt.at[idx].add(src)
def _segment_sum(src, seg, n):
    return jax.ops.segment_sum(src, seg, n)
class _Rng:
    def __init__(self, key):
        self._k = key
    def _next(self):
        self._k, sub = jax.random.split(self._k)
        return sub
    def normal(self, shape):
        return jax.random.normal(self._next(), shape, dtype=jnp.bfloat16)
    def randint(self, lo, hi, shape):
        return jax.random.randint(self._next(), shape, lo, hi, dtype=jnp.int32)
    def uniform(self, shape, lo=0.0, hi=1.0):
        return jax.random.uniform(self._next(), shape, jnp.bfloat16, lo, hi)
    def permutation(self, n):
        return jax.random.permutation(self._next(), n)


kernel_name = 'sequential_preLN__compressed_kv_cla__moe_arch_mod__decode'

def setup_inputs():
    _rng = _Rng(jax.random.key(int.from_bytes(__import__("os").urandom(4), "little")))
    _w = (lambda a: (lambda t: t.astype(jnp.bfloat16) if jnp.issubdtype(t.dtype, jnp.floating) else t)(jnp.asarray(a)))
    def _A_setup():
        B, H, Sq, Sk, D, M = 1, 32, 1, 8192, 128, 512
        Dc = 4 * D
        return {
            "x": _w((lambda *s: _rng.normal(s) * 0.05)(B, Sq, M)),
            "c_kv": _w((lambda *s: _rng.normal(s) * 0.05)(B, Sk, Dc)),
            "w_q": _w((lambda *s: _rng.normal(s) * 0.05)(M, H, D) * (M ** -0.5)),
            "w_uk": _w((lambda *s: _rng.normal(s) * 0.05)(Dc, H, D) * (Dc ** -0.5)),
            "w_uv": _w((lambda *s: _rng.normal(s) * 0.05)(Dc, H, D) * (Dc ** -0.5)),
            "w_o": _w((lambda *s: _rng.normal(s) * 0.05)(H, D, M) * ((H * D) ** -0.5)),
        }
    _A_in = _A_setup()

    def _B_setup():
        B, S, D, F, C = 1, 1, 512, 1376, 1
        return {
            "x": _w((lambda *s: _rng.normal(s) * 0.05)(B, S, D)),
            "w_r": _w((lambda *s: _rng.normal(s) * 0.05)(D)),
            "w_gate": _w((lambda *s: _rng.normal(s) * 0.05)(D, F)),
            "w_up": _w((lambda *s: _rng.normal(s) * 0.05)(D, F)),
            "w_down": _w((lambda *s: _rng.normal(s) * 0.05)(F, D)),
        }
    _B_in = _B_setup()

    return {
        "A_x": _A_in["x"],
        "A_c_kv": _A_in["c_kv"],
        "A_w_q": _A_in["w_q"],
        "A_w_uk": _A_in["w_uk"],
        "A_w_uv": _A_in["w_uv"],
        "A_w_o": _A_in["w_o"],
        "B_x": _B_in["x"],
        "B_w_r": _B_in["w_r"],
        "B_w_gate": _B_in["w_gate"],
        "B_w_up": _B_in["w_up"],
        "B_w_down": _B_in["w_down"],
    }

def reference(A_x, A_c_kv, A_w_q, A_w_uk, A_w_uv, A_w_o, B_x, B_w_r, B_w_gate, B_w_up, B_w_down):
    def _A_ref(x, c_kv, w_q, w_uk, w_uv, w_o):
        B, Sq, M = x.shape[0], x.shape[1], x.shape[2]
        Sk = c_kv.shape[1]
        H, D = w_q.shape[1], w_q.shape[2]
        q = jnp.einsum("bqm,mhd->bhqd", x, w_q)
        k = jnp.einsum("bkc,chd->bhkd", c_kv, w_uk)
        v = jnp.einsum("bkc,chd->bhkd", c_kv, w_uv)
        scores = jnp.einsum("bhqd,bhkd->bhqk", q, k) * (D ** -0.5)
        off = Sk - Sq
        qi = jnp.arange(Sq)[:, None]
        kj = jnp.arange(Sk)[None, :]
        cmask = kj <= (qi + off)
        scores = jnp.where(cmask[None, None], scores, -1e9)
        p = _softmax(scores, axis=-1)
        ctx = jnp.einsum("bhqk,bhkd->bhqd", p, v)
        return jnp.einsum("bhqd,hdm->bqm", ctx, w_o)

    def _B_ref(x, w_r, w_gate, w_up, w_down):
        B, S, D = x.shape
        C = 1
        r = x @ w_r
        idx = jnp.argsort(-r, axis=-1)[:, :C]
        idx_e = jnp.repeat(idx.reshape(B, C, 1), D, axis=2)
        x_sel = jnp.take_along_axis(x, idx_e, axis=1)
        g = _silu(x_sel @ w_gate)
        u = x_sel @ w_up
        y = (g * u) @ w_down
        r_sel = _sigmoid(jnp.take_along_axis(r, idx, axis=1))
        y = y * r_sel.reshape(B, C, 1)
        b_off = (jnp.arange(B) * S).reshape(B, 1)
        flat_idx = (idx + b_off).reshape(B * C)
        zero = (x * 0.0).reshape(B * S, D)
        upd = _scatter_add(zero, flat_idx, y.reshape(B * C, D), axis=0)
        return x + upd.reshape(B, S, D)

    x = A_x
    h = x + _A_ref(_layernorm(x, axis=-1), A_c_kv, A_w_q, A_w_uk, A_w_uv, A_w_o)
    h2 = h + _B_ref(_layernorm(h, axis=-1), B_w_r, B_w_gate, B_w_up, B_w_down)
    return h2
```

```python
import jax
import jax.numpy as jnp
from jax import lax
import jax.experimental.pallas as pl
import jax.experimental.pallas.tpu as pltpu

_EPS = 1e-5
_LANES = 128
_NT = (((1,), (1,)), ((), ()))

_KV_CHUNKS = (2048, 2048, 2048, 2048)
_DOWN_CHUNKS = (768, 384, 128, 96)


def _layernorm(x):
    m = jnp.mean(x, axis=-1, keepdims=True)
    d = x - m
    v = jnp.mean(d * d, axis=-1, keepdims=True)
    return d / jnp.sqrt(v + _EPS)


def _sigmoid(x):
    return 1.0 / (1.0 + jnp.exp(-x))


def _offsets(chunks):
    out, o = [], 0
    for n in chunks:
        out.append((o, n))
        o += n
    return out


def _kernel(x_hbm, ckv_hbm, wq_hbm, wuk_hbm, wuv_hbm, wo_hbm, wr_hbm, wg_hbm, wu_hbm, wd_hbm,
            o_ref,
            x_v, ckv_v, wq_v, wuk_v, wuv_v, wo_v, wr_v, wg_v, wu_v, wd_v, e_v, sems,
            *, heads, head_dim):
    f32, bf16 = jnp.float32, jnp.bfloat16
    H, D = heads, head_dim
    M = x_v.shape[-1]
    C = ckv_v.shape[-1]
    G = _LANES * H
    kv_chunks = _offsets(_KV_CHUNKS)
    down_chunks = _offsets(_DOWN_CHUNKS)

    copies = []

    def start(src, dst):
        cp = pltpu.make_async_copy(src, dst, sems.at[len(copies)])
        cp.start()
        copies.append(cp)
        return cp

    def start_rows(src, dst, o, n):
        return start(src.at[pl.ds(o, n)], dst.at[pl.ds(o, n)])

    cp_x = start(x_hbm, x_v)
    cp_wq = start(wq_hbm, wq_v)
    cp_wuk = start(wuk_hbm, wuk_v)
    cp_kv = [start_rows(ckv_hbm, ckv_v, o, n) for o, n in kv_chunks]
    cp_wuv = start(wuv_hbm, wuv_v)
    cp_wo = start(wo_hbm, wo_v)
    cp_wr = start(wr_hbm, wr_v)
    cp_wg = start(wg_hbm, wg_v)
    cp_wu = start(wu_hbm, wu_v)
    cp_wd = [start_rows(wd_hbm, wd_v, o, n) for o, n in down_chunks]

    rows = lax.broadcasted_iota(jnp.int32, (G, _LANES), 0)
    cols = lax.broadcasted_iota(jnp.int32, (G, _LANES), 1)
    e_v[...] = jnp.where(rows // H == cols, 1.0, 0.0).astype(bf16)
    own_head = (lax.broadcasted_iota(jnp.int32, (H, G), 1) % H
                == lax.broadcasted_iota(jnp.int32, (H, G), 0))

    def spread(coef):
        n = coef.shape[1] // _LANES
        stacked = jnp.concatenate(
            [coef[:, g * _LANES:(g + 1) * _LANES] for g in range(n)], axis=0).astype(bf16)
        rep = lax.dot_general(stacked, e_v[...], _NT, preferred_element_type=f32)
        return [jnp.where(own_head, rep[g * H:(g + 1) * H], 0.0).astype(bf16) for g in range(n)]

    def per_head_matvec(lhs, w_ref):
        acc = None
        for g, l in enumerate(lhs):
            t = jnp.dot(l, w_ref[pl.ds(g * G, G), :], preferred_element_type=f32)
            acc = t if acc is None else acc + t
        return acc

    cp_x.wait()
    x = x_v[0].astype(f32)
    xn = _layernorm(x)
    lhs_q = spread(jnp.broadcast_to(xn, (H, M)))
    cp_wq.wait()
    q = per_head_matvec(lhs_q, wq_v).astype(bf16)

    cp_wuk.wait()
    picked = []
    for g in range(C // _LANES):
        s = lax.dot_general(q, wuk_v[pl.ds(g * G, G), :], _NT, preferred_element_type=f32)
        picked.append(jnp.where(own_head, s * (D ** -0.5), 0.0).astype(bf16))
    qa = jnp.dot(jnp.concatenate(picked, axis=0), e_v[...], preferred_element_type=f32)
    qa = jnp.concatenate([qa[g * H:(g + 1) * H] for g in range(C // _LANES)], axis=1).astype(bf16)

    m = l = acc = None
    for cp, (o, n) in zip(cp_kv, kv_chunks):
        cp.wait()
        c = ckv_v[pl.ds(o, n), :]
        s = lax.dot_general(qa, c, _NT, preferred_element_type=f32)
        m_blk = jnp.max(s, axis=-1, keepdims=True)
        m_new = m_blk if m is None else jnp.maximum(m, m_blk)
        p = jnp.exp(s - m_new)
        l_blk = jnp.sum(p, axis=-1, keepdims=True)
        pv = jnp.dot(p.astype(bf16), c, preferred_element_type=f32)
        if m is None:
            l, acc = l_blk, pv
        else:
            alpha = jnp.exp(m - m_new)
            l, acc = alpha * l + l_blk, alpha * acc + pv
        m = m_new
    lhs_v = spread(acc / l)

    cp_wuv.wait()
    ctx = per_head_matvec(lhs_v, wuv_v)

    sub = lax.broadcasted_iota(jnp.int32, (8, D), 0)
    lhs_o = jnp.concatenate(
        [jnp.where(sub == h % 8, ctx[h // 8 * 8:h // 8 * 8 + 8], 0.0) for h in range(H)],
        axis=1).astype(bf16)
    cp_wo.wait()
    attn = jnp.sum(jnp.dot(lhs_o, wo_v[...], preferred_element_type=f32), axis=0, keepdims=True)
    h1 = x + attn
    hn = _layernorm(h1)

    hb = jnp.broadcast_to(hn, (8, M)).astype(bf16)
    cp_wr.wait()
    wr = wr_v[...].astype(f32)
    r = sum(jnp.sum(hn[:, i * _LANES:(i + 1) * _LANES] * wr[i:i + 1], axis=-1, keepdims=True)
            for i in range(M // _LANES))
    gate_r = _sigmoid(r)
    cp_wg.wait()
    gt = lax.dot_general(hb, wg_v[...], _NT, preferred_element_type=f32)
    gt = gt * _sigmoid(gt)
    cp_wu.wait()
    up = lax.dot_general(hb, wu_v[...], _NT, preferred_element_type=f32)
    act = (gt * up).astype(bf16)
    y = None
    for cp, (o, n) in zip(cp_wd, down_chunks):
        cp.wait()
        t = jnp.dot(act[:, o:o + n], wd_v[pl.ds(o, n), :], preferred_element_type=f32)
        y = t if y is None else y + t
    upd = hn * 0.0 + y[0:1] * gate_r
    o_ref[0] = (h1 + (hn + upd)).astype(o_ref.dtype)


@jax.jit
def pallas_sequential_preLN__compressed_kv_cla__moe_arch_mod__decode_kernel(
    A_x: jax.Array,
    A_c_kv: jax.Array,
    A_w_q: jax.Array,
    A_w_uk: jax.Array,
    A_w_uv: jax.Array,
    A_w_o: jax.Array,
    B_x: jax.Array,
    B_w_r: jax.Array,
    B_w_gate: jax.Array,
    B_w_up: jax.Array,
    B_w_down: jax.Array,
):
    del B_x
    B, Sq, M = A_x.shape
    _, Sk, C = A_c_kv.shape
    _, H, D = A_w_q.shape
    F = B_w_gate.shape[1]
    assert B == 1 and Sq == 1 and D == _LANES
    assert sum(_KV_CHUNKS) == Sk and sum(_DOWN_CHUNKS) == F
    bf16 = jnp.bfloat16

    operands = (
        A_x,
        A_c_kv.reshape(Sk, C),
        A_w_q.reshape(M * H, D),
        A_w_uk.reshape(C * H, D),
        A_w_uv.reshape(C * H, D),
        A_w_o.reshape(H * D, M),
        B_w_r.reshape(M // _LANES, _LANES),
        B_w_gate.T,
        B_w_up.T,
        B_w_down,
    )
    n_copies = 8 + len(_KV_CHUNKS) + len(_DOWN_CHUNKS)

    def body(*refs):
        _kernel(*refs, heads=H, head_dim=D)

    return pl.pallas_call(
        body,
        in_specs=[pl.BlockSpec(memory_space=pltpu.HBM)] * len(operands),
        out_specs=pl.BlockSpec(memory_space=pltpu.VMEM),
        out_shape=jax.ShapeDtypeStruct((B, Sq, M), A_x.dtype),
        scratch_shapes=[pltpu.VMEM(a.shape, a.dtype) for a in operands] + [
            pltpu.VMEM((_LANES * H, _LANES), bf16),
            pltpu.SemaphoreType.DMA((n_copies,)),
        ],
        compiler_params=pltpu.CompilerParams(vmem_limit_bytes=96 * 1024 * 1024),
    )(*operands)
```

```python
import jax
import jax.numpy as jnp
from jax import lax
import jax.experimental.pallas as pl
import jax.experimental.pallas.tpu as pltpu

_EPS = 1e-5
_LANES = 128
_NT = (((1,), (1,)), ((), ()))

_HEAD_ROWS = 512
_KV_ROWS = 256
_OUT_ROWS = 128
_FFN_CHUNKS = (128,) * 9 + (224,)
_DOWN_CHUNKS = (128,) * 5 + (48,)
_PIECE_BYTES = 32 * 1024
_LOOKAHEAD = 96
_FIRST_QUEUE = 1
_FLOOR = False


class _Stream:
    def __init__(self, sems):
        self.sems = sems
        self.pieces = []
        self.steps = []
        self.issued = 0

    def add(self, *blocks):
        lanes, waits = [], []
        for k, (src, dst, *rows) in enumerate(blocks):
            sem = 2 * len(self.steps) + k
            queue = (k + _FIRST_QUEUE) % 2
            if rows:
                lo, n = rows
                step = _PIECE_BYTES // (dst.shape[1] * dst.dtype.itemsize)
                cuts = [pl.ds(o, min(step, lo + n - o)) for o in range(lo, lo + n, step)]
                lanes.append([(src.at[c], dst.at[c], sem, queue) for c in cuts])
                waits.append((dst.at[pl.ds(lo, n)], sem))
            else:
                lanes.append([(src, dst, sem, queue)])
                waits.append((dst, sem))
        for i in range(max(len(lane) for lane in lanes)):
            self.pieces += [lane[i] for lane in lanes if i < len(lane)]
        self.steps.append((waits, len(self.pieces)))
        return len(self.steps) - 1

    def add_halves(self, src, dst, rows):
        half = dst.shape[0] // 2
        return [(self.add((src, dst, o, rows), (src, dst, half + o, rows)), (o, half + o))
                for o in range(0, half, rows)]

    def issue(self, upto):
        upto = min(upto, len(self.pieces))
        for src, dst, sem, queue in self.pieces[self.issued:upto]:
            pltpu.make_async_copy(src, dst, self.sems.at[sem]).start(priority=queue)
        self.issued = max(self.issued, upto)

    def wait(self, step):
        waits, end = self.steps[step]
        self.issue(end + _LOOKAHEAD)
        for dst, sem in waits:
            pltpu.make_async_copy(dst, dst, self.sems.at[sem]).wait()


def _layernorm(x):
    m = jnp.mean(x, axis=-1, keepdims=True)
    d = x - m
    v = jnp.mean(d * d, axis=-1, keepdims=True)
    return d / jnp.sqrt(v + _EPS)


def _sigmoid(x):
    return 1.0 / (1.0 + jnp.exp(-x))


def _kernel(x_hbm, ckv_hbm, wq_hbm, wuk_hbm, wuv_hbm, wo_hbm, wr_hbm, wg_hbm, wu_hbm, wd_hbm,
            o_ref,
            x_v, ckv_v, wq_v, wuk_v, wuv_v, wo_v, wr_v, wg_v, wu_v, wd_v, e_v, sems,
            *, heads, head_dim):
    f32, bf16 = jnp.float32, jnp.bfloat16
    H, D = heads, head_dim
    M = x_v.shape[-1]
    C = ckv_v.shape[-1]
    G = _LANES * H
    F = wd_v.shape[0]

    stream = _Stream(sems)
    s_x = stream.add((x_hbm, x_v), (wr_hbm, wr_v))
    s_wq = stream.add_halves(wq_hbm, wq_v, _HEAD_ROWS)
    s_wuk = stream.add_halves(wuk_hbm, wuk_v, _HEAD_ROWS)
    s_kv = stream.add_halves(ckv_hbm, ckv_v, _KV_ROWS)
    s_wuv = stream.add_halves(wuv_hbm, wuv_v, _HEAD_ROWS)
    s_wo = stream.add_halves(wo_hbm, wo_v, _OUT_ROWS)
    s_ffn, o = [], 0
    for n in _FFN_CHUNKS:
        s_ffn.append((stream.add((wg_hbm, wg_v, o, n), (wu_hbm, wu_v, o, n)), o, n))
        o += n
    s_down, o, half = [], 0, sum(_DOWN_CHUNKS[:-1])
    for n in _DOWN_CHUNKS[:-1]:
        s_down.append((stream.add((wd_hbm, wd_v, o, n), (wd_hbm, wd_v, half + o, n)),
                       ((o, n), (half + o, n))))
        o += n
    n = _DOWN_CHUNKS[-1]
    s_down.append((stream.add((wd_hbm, wd_v, 2 * half, n), (wd_hbm, wd_v, 2 * half + n, n)),
                   ((2 * half, 2 * n),)))
    stream.issue(_LOOKAHEAD)
    if _FLOOR:
        for b in range(len(stream.steps)):
            stream.wait(b)
        o_ref[0] = x_v[0]
        return

    rows = lax.broadcasted_iota(jnp.int32, (G, _LANES), 0)
    cols = lax.broadcasted_iota(jnp.int32, (G, _LANES), 1)
    e_v[...] = jnp.where(rows // H == cols, 1.0, 0.0).astype(bf16)
    own_head = (lax.broadcasted_iota(jnp.int32, (H, G), 1) % H
                == lax.broadcasted_iota(jnp.int32, (H, G), 0))

    def spread(coef):
        n = coef.shape[1] // _LANES
        stacked = jnp.concatenate(
            [coef[:, g * _LANES:(g + 1) * _LANES] for g in range(n)], axis=0).astype(bf16)
        rep = lax.dot_general(stacked, e_v[...], _NT, preferred_element_type=f32)
        return [jnp.where(own_head, rep[g * H:(g + 1) * H], 0.0).astype(bf16) for g in range(n)]

    def per_head_matvec(lhs, w_ref, steps):
        acc = None
        for step, offsets in steps:
            stream.wait(step)
            for o in offsets:
                t = jnp.dot(lhs[o // G][:, o % G:o % G + _HEAD_ROWS],
                            w_ref[pl.ds(o, _HEAD_ROWS), :], preferred_element_type=f32)
                acc = t if acc is None else acc + t
        return acc

    stream.wait(s_x)
    x = x_v[0].astype(f32)
    xn = _layernorm(x)
    lhs_q = spread(jnp.broadcast_to(xn, (H, M)))
    q = per_head_matvec(lhs_q, wq_v, s_wq).astype(bf16)

    picked = {}
    for step, offsets in s_wuk:
        stream.wait(step)
        for o in offsets:
            s = lax.dot_general(q, wuk_v[pl.ds(o, _HEAD_ROWS), :], _NT, preferred_element_type=f32)
            picked[o] = jnp.where(own_head[:, :_HEAD_ROWS], s * (D ** -0.5), 0.0).astype(bf16)
    picked = [jnp.concatenate([picked[o] for o in range(g, g + G, _HEAD_ROWS)], axis=1)
              for g in range(0, C * H, G)]
    qa = jnp.dot(jnp.concatenate(picked, axis=0), e_v[...], preferred_element_type=f32)
    qa = jnp.concatenate([qa[g * H:(g + 1) * H] for g in range(C // _LANES)], axis=1).astype(bf16)

    m = l = acc = None
    for step, offsets in s_kv:
        stream.wait(step)
        c = jnp.concatenate([ckv_v[pl.ds(o, _KV_ROWS), :] for o in offsets], axis=0)
        s = lax.dot_general(qa, c, _NT, preferred_element_type=f32)
        m_blk = jnp.max(s, axis=-1, keepdims=True)
        m_new = m_blk if m is None else jnp.maximum(m, m_blk)
        p = jnp.exp(s - m_new)
        l_blk = jnp.sum(p, axis=-1, keepdims=True)
        pv = jnp.dot(p.astype(bf16), c, preferred_element_type=f32)
        if m is None:
            l, acc = l_blk, pv
        else:
            alpha = jnp.exp(m - m_new)
            l, acc = alpha * l + l_blk, alpha * acc + pv
        m = m_new
    lhs_v = spread(acc / l)

    ctx = per_head_matvec(lhs_v, wuv_v, s_wuv)

    sub = lax.broadcasted_iota(jnp.int32, (8, D), 0)
    lhs_o = jnp.concatenate(
        [jnp.where(sub == h % 8, ctx[h // 8 * 8:h // 8 * 8 + 8], 0.0) for h in range(H)],
        axis=1).astype(bf16)
    attn = None
    for step, offsets in s_wo:
        stream.wait(step)
        for o in offsets:
            t = jnp.dot(lhs_o[:, o:o + _OUT_ROWS], wo_v[pl.ds(o, _OUT_ROWS), :],
                        preferred_element_type=f32)
            attn = t if attn is None else attn + t
    attn = jnp.sum(attn, axis=0, keepdims=True)
    h1 = x + attn
    hn = _layernorm(h1)

    hb = jnp.broadcast_to(hn, (8, M)).astype(bf16)
    wr = wr_v[...].astype(f32)
    r = sum(jnp.sum(hn[:, i * _LANES:(i + 1) * _LANES] * wr[i:i + 1], axis=-1, keepdims=True)
            for i in range(M // _LANES))
    gate_r = _sigmoid(r)

    act = []
    for step, o, n in s_ffn:
        stream.wait(step)
        gt = lax.dot_general(hb, wg_v[pl.ds(o, n), :], _NT, preferred_element_type=f32)
        up = lax.dot_general(hb, wu_v[pl.ds(o, n), :], _NT, preferred_element_type=f32)
        act.append((gt * _sigmoid(gt) * up).astype(bf16))
    act = jnp.concatenate(act, axis=1)
    y = None
    for step, blocks in s_down:
        stream.wait(step)
        for o, n in blocks:
            t = jnp.dot(act[:, o:o + n], wd_v[pl.ds(o, n), :], preferred_element_type=f32)
            y = t if y is None else y + t
    upd = hn * 0.0 + y[0:1] * gate_r
    o_ref[0] = (h1 + (hn + upd)).astype(o_ref.dtype)


@jax.jit
def pallas_sequential_preLN__compressed_kv_cla__moe_arch_mod__decode_kernel(
    A_x: jax.Array,
    A_c_kv: jax.Array,
    A_w_q: jax.Array,
    A_w_uk: jax.Array,
    A_w_uv: jax.Array,
    A_w_o: jax.Array,
    B_x: jax.Array,
    B_w_r: jax.Array,
    B_w_gate: jax.Array,
    B_w_up: jax.Array,
    B_w_down: jax.Array,
):
    del B_x
    B, Sq, M = A_x.shape
    _, Sk, C = A_c_kv.shape
    _, H, D = A_w_q.shape
    F = B_w_gate.shape[1]
    assert B == 1 and Sq == 1 and D == _LANES
    assert sum(_FFN_CHUNKS) == F and 2 * sum(_DOWN_CHUNKS) == F and M == C
    bf16 = jnp.bfloat16

    operands = (
        A_x,
        A_c_kv.reshape(Sk, C),
        A_w_q.reshape(M * H, D),
        A_w_uk.reshape(C * H, D),
        A_w_uv.reshape(C * H, D),
        A_w_o.reshape(H * D, M),
        B_w_r.reshape(M // _LANES, _LANES),
        B_w_gate.T,
        B_w_up.T,
        B_w_down,
    )
    n_copies = (2 + (M + 2 * C) * H // _HEAD_ROWS + Sk // _KV_ROWS + H * D // _OUT_ROWS
                + 2 * len(_FFN_CHUNKS) + 2 * len(_DOWN_CHUNKS))

    def body(*refs):
        pl.run_scoped(lambda sems: _kernel(*refs, sems, heads=H, head_dim=D),
                      pltpu.SemaphoreType.DMA((n_copies,)))

    return pl.pallas_call(
        body,
        in_specs=[pl.BlockSpec(memory_space=pltpu.HBM)] * len(operands),
        out_specs=pl.BlockSpec(memory_space=pltpu.VMEM),
        out_shape=jax.ShapeDtypeStruct((B, Sq, M), A_x.dtype),
        scratch_shapes=[pltpu.VMEM(a.shape, a.dtype) for a in operands] + [
            pltpu.VMEM((_LANES * H, _LANES), bf16)],
        compiler_params=pltpu.CompilerParams(vmem_limit_bytes=96 * 1024 * 1024),
    )(*operands)
```

```python
import jax
import jax.numpy as jnp
from jax import lax
import jax.experimental.pallas as pl
import jax.experimental.pallas.tpu as pltpu

_EPS = 1e-5
_LANES = 128
_NT = (((1,), (1,)), ((), ()))

_HEAD_ROWS = 512
_KV_ROWS = 256
_OUT_ROWS = 128
_FFN_CHUNKS = (128,) * 9
_DOWN_EARLY = 640
_DOWN_MXU = (256, 256)
_DOWN_VPU = (128, 64, 32)
_PIN = True
_PIECE_BYTES = 32 * 1024
_LOOKAHEAD = 96
_FLOOR = False


class _Stream:
    def __init__(self, sems):
        self.sems = sems
        self.pieces = []
        self.blocks = []
        self.ends = {}
        self.issued = 0

    def add(self, slow, fast):
        lanes, ids = [], []
        for queue, blocks in ((1, slow), (0, fast)):
            lanes.append([])
            ids.append([])
            for src, dst, *rows in blocks:
                if rows:
                    lo, n = rows
                    step = _PIECE_BYTES // (dst.shape[1] * dst.dtype.itemsize)
                    cuts = [pl.ds(o, min(step, lo + n - o)) for o in range(lo, lo + n, step)]
                    parts = [(src.at[c], dst.at[c]) for c in cuts]
                    dst = dst.at[pl.ds(lo, n)]
                else:
                    parts = [(src, dst)]
                lanes[-1] += [part + (len(self.blocks), queue) for part in parts]
                ids[-1].append(len(self.blocks))
                self.blocks.append(dst)
        for i in range(max(len(lane) for lane in lanes)):
            for lane in lanes:
                if i < len(lane):
                    self.pieces.append(lane[i])
                    self.ends[lane[i][2]] = len(self.pieces)
        return ids

    def add_halves(self, src, dst, rows):
        half = dst.shape[0] // 2
        starts = range(0, half, rows)
        slow, fast = self.add([(src, dst, o, rows) for o in starts],
                              [(src, dst, half + o, rows) for o in starts])
        return [((a, b), (o, half + o)) for a, b, o in zip(slow, fast, starts)]

    def issue(self, upto):
        upto = min(upto, len(self.pieces))
        for src, dst, block, queue in self.pieces[self.issued:upto]:
            pltpu.make_async_copy(src, dst, self.sems.at[block]).start(priority=queue)
        self.issued = max(self.issued, upto)

    def wait(self, *blocks):
        self.issue(max(self.ends[b] for b in blocks) + _LOOKAHEAD)
        for b in blocks:
            pltpu.make_async_copy(self.blocks[b], self.blocks[b], self.sems.at[b]).wait()


def _layernorm(x):
    m = jnp.mean(x, axis=-1, keepdims=True)
    d = x - m
    v = jnp.mean(d * d, axis=-1, keepdims=True)
    return d / jnp.sqrt(v + _EPS)


def _sigmoid(x):
    return 1.0 / (1.0 + jnp.exp(-x))


def _consecutive(start, sizes):
    out = []
    for n in sizes:
        out.append((start, n))
        start += n
    return out


def _kernel(x_hbm, ckv_hbm, wq_hbm, wuk_hbm, wuv_hbm, wo_hbm, wr_hbm, wg_hbm, wu_hbm, wd_hbm,
            o_ref,
            x_v, ckv_v, wq_v, wuk_v, wuv_v, wo_v, wr_v, wg_v, wu_v, wd_v, e_v, y_v, sems,
            *, heads, head_dim):
    f32, bf16 = jnp.float32, jnp.bfloat16
    H, D = heads, head_dim
    M = x_v.shape[-1]
    C = ckv_v.shape[-1]
    G = _LANES * H
    F = wd_v.shape[0]

    stream = _Stream(sems)
    (b_x,), (b_wr,) = stream.add([(x_hbm, x_v)], [(wr_hbm, wr_v)])
    s_wq = stream.add_halves(wq_hbm, wq_v, _HEAD_ROWS)
    s_wuk = stream.add_halves(wuk_hbm, wuk_v, _HEAD_ROWS)
    s_kv = stream.add_halves(ckv_hbm, ckv_v, _KV_ROWS)
    s_wuv = stream.add_halves(wuv_hbm, wuv_v, _HEAD_ROWS)
    s_wo = stream.add_halves(wo_hbm, wo_v, _OUT_ROWS)
    vpu_rows = (F - sum(_DOWN_VPU), sum(_DOWN_VPU))
    ffn_rows = [vpu_rows] + _consecutive(0, _FFN_CHUNKS)
    b_gate, b_up = stream.add([(wg_hbm, wg_v, *r) for r in ffn_rows],
                              [(wu_hbm, wu_v, *r) for r in ffn_rows])
    down_rows = _consecutive(_DOWN_EARLY, _DOWN_MXU + _DOWN_VPU)
    b_down, b_early = stream.add([(wd_hbm, wd_v, *r) for r in down_rows],
                                 [(wd_hbm, wd_v, 0, _DOWN_EARLY)])
    stream.issue(_LOOKAHEAD)
    if _FLOOR:
        for b in range(len(stream.blocks)):
            stream.wait(b)
        o_ref[0] = x_v[0]
        return

    rows = lax.broadcasted_iota(jnp.int32, (G, _LANES), 0)
    cols = lax.broadcasted_iota(jnp.int32, (G, _LANES), 1)
    e_v[...] = jnp.where(rows // H == cols, 1.0, 0.0).astype(bf16)
    own_head = (lax.broadcasted_iota(jnp.int32, (H, G), 1) % H
                == lax.broadcasted_iota(jnp.int32, (H, G), 0))

    def spread(coef):
        n = coef.shape[1] // _LANES
        stacked = jnp.concatenate(
            [coef[:, g * _LANES:(g + 1) * _LANES] for g in range(n)], axis=0).astype(bf16)
        rep = lax.dot_general(stacked, e_v[...], _NT, preferred_element_type=f32)
        return [jnp.where(own_head, rep[g * H:(g + 1) * H], 0.0).astype(bf16) for g in range(n)]

    def per_head_matvec(lhs, w_ref, steps):
        acc = None
        for step, offsets in steps:
            stream.wait(*step)
            for o in offsets:
                t = jnp.dot(lhs[o // G][:, o % G:o % G + _HEAD_ROWS],
                            w_ref[pl.ds(o, _HEAD_ROWS), :], preferred_element_type=f32)
                acc = t if acc is None else acc + t
        return acc

    stream.wait(b_x, b_wr)
    x = x_v[0].astype(f32)
    xn = _layernorm(x)
    lhs_q = spread(jnp.broadcast_to(xn, (H, M)))
    q = per_head_matvec(lhs_q, wq_v, s_wq).astype(bf16)

    picked = {}
    for step, offsets in s_wuk:
        stream.wait(*step)
        for o in offsets:
            s = lax.dot_general(q, wuk_v[pl.ds(o, _HEAD_ROWS), :], _NT, preferred_element_type=f32)
            picked[o] = jnp.where(own_head[:, :_HEAD_ROWS], s * (D ** -0.5), 0.0).astype(bf16)
    picked = [jnp.concatenate([picked[o] for o in range(g, g + G, _HEAD_ROWS)], axis=1)
              for g in range(0, C * H, G)]
    qa = jnp.dot(jnp.concatenate(picked, axis=0), e_v[...], preferred_element_type=f32)
    qa = jnp.concatenate([qa[g * H:(g + 1) * H] for g in range(C // _LANES)], axis=1).astype(bf16)

    m = l = acc = None
    for step, offsets in s_kv:
        stream.wait(*step)
        c = jnp.concatenate([ckv_v[pl.ds(o, _KV_ROWS), :] for o in offsets], axis=0)
        s = lax.dot_general(qa, c, _NT, preferred_element_type=f32)
        m_blk = jnp.max(s, axis=-1, keepdims=True)
        m_new = m_blk if m is None else jnp.maximum(m, m_blk)
        p = jnp.exp(s - m_new)
        l_blk = jnp.sum(p, axis=-1, keepdims=True)
        pv = jnp.dot(p.astype(bf16), c, preferred_element_type=f32)
        if m is None:
            l, acc = l_blk, pv
        else:
            alpha = jnp.exp(m - m_new)
            l, acc = alpha * l + l_blk, alpha * acc + pv
        m = m_new
    lhs_v = spread(acc / l)

    ctx = per_head_matvec(lhs_v, wuv_v, s_wuv)

    sub = lax.broadcasted_iota(jnp.int32, (8, D), 0)
    lhs_o = jnp.concatenate(
        [jnp.where(sub == h % 8, ctx[h // 8 * 8:h // 8 * 8 + 8], 0.0) for h in range(H)],
        axis=1).astype(bf16)
    attn = None
    for step, offsets in s_wo:
        stream.wait(*step)
        for o in offsets:
            t = jnp.dot(lhs_o[:, o:o + _OUT_ROWS], wo_v[pl.ds(o, _OUT_ROWS), :],
                        preferred_element_type=f32)
            attn = t if attn is None else attn + t
    attn = jnp.sum(attn, axis=0, keepdims=True)
    h1 = x + attn
    hn = _layernorm(h1)

    hb = jnp.broadcast_to(hn, (_LANES, M)).astype(bf16)
    wr = wr_v[...].astype(f32)
    r = sum(jnp.sum(hn[:, i * _LANES:(i + 1) * _LANES] * wr[i:i + 1], axis=-1, keepdims=True)
            for i in range(M // _LANES))
    route = _sigmoid(r)
    act = []
    for bg, bu, (o, n) in zip(b_gate, b_up, ffn_rows):
        stream.wait(bg, bu)
        wg, wu = wg_v[pl.ds(o, n), :], wu_v[pl.ds(o, n), :]
        if act:
            gt = lax.dot_general(hb[:8], wg, _NT, preferred_element_type=f32)
            up = lax.dot_general(hb[:8], wu, _NT, preferred_element_type=f32)
        else:
            gt = lax.dot_general(wg, hb, _NT, preferred_element_type=f32)
            up = lax.dot_general(wu, hb, _NT, preferred_element_type=f32)
        act.append(gt * _sigmoid(gt) * up * route)
    act_col = act[0]
    act = jnp.concatenate(act[1:], axis=1).astype(bf16)

    first = lax.broadcasted_iota(jnp.int32, (8, M), 0) == 0
    y_v[...] = jnp.where(first, h1 + (hn + hn * 0.0), 0.0)
    for b, (o, n) in zip(b_early + b_down, [(0, _DOWN_EARLY)] + down_rows):
        stream.wait(b)
        w = wd_v[pl.ds(o, n), :]
        if o < vpu_rows[0]:
            t = jnp.where(first, jnp.dot(act[:, o:o + n], w, preferred_element_type=f32), 0.0)
        else:
            a = act_col[o - vpu_rows[0]:o - vpu_rows[0] + n]
            t = w.astype(f32) * jnp.concatenate([a] * (M // _LANES), axis=1)
            t = jnp.sum(t.reshape(n // 8, 8, M), axis=0)
        if o + n < F and _PIN:
            y_v[...] += t
        elif _PIN:
            o_ref[0] = jnp.sum(y_v[...] + t, axis=0, keepdims=True).astype(o_ref.dtype)
        else:
            y = (y_v[...] if o == 0 else y) + t
    if not _PIN:
        o_ref[0] = jnp.sum(y, axis=0, keepdims=True).astype(o_ref.dtype)


@jax.jit
def pallas_sequential_preLN__compressed_kv_cla__moe_arch_mod__decode_kernel(
    A_x: jax.Array,
    A_c_kv: jax.Array,
    A_w_q: jax.Array,
    A_w_uk: jax.Array,
    A_w_uv: jax.Array,
    A_w_o: jax.Array,
    B_x: jax.Array,
    B_w_r: jax.Array,
    B_w_gate: jax.Array,
    B_w_up: jax.Array,
    B_w_down: jax.Array,
):
    del B_x
    B, Sq, M = A_x.shape
    _, Sk, C = A_c_kv.shape
    _, H, D = A_w_q.shape
    F = B_w_gate.shape[1]
    assert B == 1 and Sq == 1 and D == _LANES
    assert M == C and sum(_FFN_CHUNKS) + sum(_DOWN_VPU) == F
    assert _DOWN_EARLY + sum(_DOWN_MXU) == sum(_FFN_CHUNKS)
    bf16 = jnp.bfloat16

    operands = (
        A_x,
        A_c_kv.reshape(Sk, C),
        A_w_q.reshape(M * H, D),
        A_w_uk.reshape(C * H, D),
        A_w_uv.reshape(C * H, D),
        A_w_o.reshape(H * D, M),
        B_w_r.reshape(M // _LANES, _LANES),
        B_w_gate.T,
        B_w_up.T,
        B_w_down,
    )
    n_copies = (2 + (M + 2 * C) * H // _HEAD_ROWS + Sk // _KV_ROWS + H * D // _OUT_ROWS
                + 2 * (1 + len(_FFN_CHUNKS)) + 1 + len(_DOWN_MXU) + len(_DOWN_VPU))

    def body(*refs):
        pl.run_scoped(lambda sems: _kernel(*refs, sems, heads=H, head_dim=D),
                      pltpu.SemaphoreType.DMA((n_copies,)))

    return pl.pallas_call(
        body,
        in_specs=[pl.BlockSpec(memory_space=pltpu.HBM)] * len(operands),
        out_specs=pl.BlockSpec(memory_space=pltpu.VMEM),
        out_shape=jax.ShapeDtypeStruct((B, Sq, M), A_x.dtype),
        scratch_shapes=[pltpu.VMEM(a.shape, a.dtype) for a in operands] + [
            pltpu.VMEM((_LANES * H, _LANES), bf16),
            pltpu.VMEM((8, M), jnp.float32)],
        compiler_params=pltpu.CompilerParams(vmem_limit_bytes=96 * 1024 * 1024),
    )(*operands)
```

```python
import jax
import jax.numpy as jnp
from jax import lax
import jax.experimental.pallas as pl
import jax.experimental.pallas.tpu as pltpu

_EPS = 1e-5
_LANES = 128
_NT = (((1,), (1,)), ((), ()))

_HEAD_ROWS = 512
_KV_ROWS = 256
_OUT_ROWS = 128
_FFN_CHUNKS = (128,) * 9
_DOWN_EARLY = 640
_DOWN_MXU = (256, 256)
_DOWN_VPU = (128, 64, 32)
_PIN = True
_TAIL_BYTES = 32 * 1024
_START_STEPS = 4
_START_BYTES = 8192
_FIRST_ISSUE = 210
_SECOND_ISSUE = 225
_PIECE_BYTES = 32 * 1024
_LOOKAHEAD = 96
_FLOOR = False


class _Stream:
    def __init__(self, sems):
        self.sems = sems
        self.pieces = []
        self.blocks = []
        self.ends = {}
        self.issued = 0

    def add(self, slow, fast, piece_bytes=None):
        lanes, ids = [], []
        for queue, blocks in ((1, slow), (0, fast)):
            lanes.append([])
            ids.append([])
            for src, dst, *rows in blocks:
                if rows:
                    lo, n = rows
                    step = (piece_bytes or _PIECE_BYTES) // (dst.shape[1] * dst.dtype.itemsize)
                    cuts = [pl.ds(o, min(step, lo + n - o)) for o in range(lo, lo + n, step)]
                    parts = [(src.at[c], dst.at[c]) for c in cuts]
                    dst = dst.at[pl.ds(lo, n)]
                else:
                    parts = [(src, dst)]
                lanes[-1] += [part + (len(self.blocks), queue) for part in parts]
                ids[-1].append(len(self.blocks))
                self.blocks.append(dst)
        for i in range(max(len(lane) for lane in lanes)):
            for lane in lanes:
                if i < len(lane):
                    self.pieces.append(lane[i])
                    self.ends[lane[i][2]] = len(self.pieces)
        return ids

    def add_halves(self, src, dst, rows, small=0):
        half = dst.shape[0] // 2
        starts = range(0, half, rows)
        slow, fast = [], []
        for part, size in ((starts[:small], _START_BYTES), (starts[small:], None)):
            a, b = self.add([(src, dst, o, rows) for o in part],
                            [(src, dst, half + o, rows) for o in part], size)
            slow, fast = slow + a, fast + b
        return [((a, b), (o, half + o)) for a, b, o in zip(slow, fast, starts)]

    def issue(self, upto):
        upto = min(upto, len(self.pieces))
        for src, dst, block, queue in self.pieces[self.issued:upto]:
            pltpu.make_async_copy(src, dst, self.sems.at[block]).start(priority=queue)
        self.issued = max(self.issued, upto)

    def wait(self, *blocks):
        self.issue(max(self.ends[b] for b in blocks) + _LOOKAHEAD)
        for b in blocks:
            pltpu.make_async_copy(self.blocks[b], self.blocks[b], self.sems.at[b]).wait()


def _layernorm(x):
    m = jnp.mean(x, axis=-1, keepdims=True)
    d = x - m
    v = jnp.mean(d * d, axis=-1, keepdims=True)
    return d / jnp.sqrt(v + _EPS)


def _sigmoid(x):
    return 1.0 / (1.0 + jnp.exp(-x))


def _consecutive(start, sizes):
    out = []
    for n in sizes:
        out.append((start, n))
        start += n
    return out


def _kernel(x_hbm, ckv_hbm, wq_hbm, wuk_hbm, wuv_hbm, wo_hbm, wr_hbm, wg_hbm, wu_hbm, wd_hbm,
            o_ref,
            x_v, ckv_v, wq_v, wuk_v, wuv_v, wo_v, wr_v, wg_v, wu_v, wd_v, e_v, y_v, sems,
            *, heads, head_dim):
    f32, bf16 = jnp.float32, jnp.bfloat16
    H, D = heads, head_dim
    M = x_v.shape[-1]
    C = ckv_v.shape[-1]
    G = _LANES * H
    F = wd_v.shape[0]

    stream = _Stream(sems)
    (b_x,), (b_wr,) = stream.add([(x_hbm, x_v)], [(wr_hbm, wr_v)])
    s_wq = stream.add_halves(wq_hbm, wq_v, _HEAD_ROWS, _START_STEPS)
    s_wuk = stream.add_halves(wuk_hbm, wuk_v, _HEAD_ROWS)
    s_kv = stream.add_halves(ckv_hbm, ckv_v, _KV_ROWS)
    s_wuv = stream.add_halves(wuv_hbm, wuv_v, _HEAD_ROWS)
    s_wo = stream.add_halves(wo_hbm, wo_v, _OUT_ROWS)
    vpu_rows = (F - sum(_DOWN_VPU), sum(_DOWN_VPU))
    ffn_rows = [vpu_rows] + _consecutive(0, _FFN_CHUNKS)
    b_gate, b_up = stream.add([(wg_hbm, wg_v, *r) for r in ffn_rows],
                              [(wu_hbm, wu_v, *r) for r in ffn_rows])
    down_rows = _consecutive(_DOWN_EARLY, _DOWN_MXU + _DOWN_VPU)
    b_down, b_early = stream.add([(wd_hbm, wd_v, *r) for r in down_rows],
                                 [(wd_hbm, wd_v, 0, _DOWN_EARLY)], _TAIL_BYTES)
    stream.issue(_FIRST_ISSUE)
    if _FLOOR:
        for b in range(len(stream.blocks)):
            stream.wait(b)
        o_ref[0] = x_v[0]
        return

    rows = lax.broadcasted_iota(jnp.int32, (G, _LANES), 0)
    cols = lax.broadcasted_iota(jnp.int32, (G, _LANES), 1)
    e_v[...] = jnp.where(rows // H == cols, 1.0, 0.0).astype(bf16)
    own_head = (lax.broadcasted_iota(jnp.int32, (H, G), 1) % H
                == lax.broadcasted_iota(jnp.int32, (H, G), 0))

    def spread(coef):
        n = coef.shape[1] // _LANES
        stacked = jnp.concatenate(
            [coef[:, g * _LANES:(g + 1) * _LANES] for g in range(n)], axis=0).astype(bf16)
        rep = lax.dot_general(stacked, e_v[...], _NT, preferred_element_type=f32)
        return [jnp.where(own_head, rep[g * H:(g + 1) * H], 0.0).astype(bf16) for g in range(n)]

    def per_head_matvec(lhs, w_ref, steps):
        acc = None
        for step, offsets in steps:
            stream.wait(*step)
            for o in offsets:
                t = jnp.dot(lhs[o // G][:, o % G:o % G + _HEAD_ROWS],
                            w_ref[pl.ds(o, _HEAD_ROWS), :], preferred_element_type=f32)
                acc = t if acc is None else acc + t
        return acc

    stream.issue(_SECOND_ISSUE)
    stream.wait(b_x, b_wr)
    x = x_v[0].astype(f32)
    xn = _layernorm(x)
    lhs_q = spread(jnp.broadcast_to(xn, (H, M)))
    q = per_head_matvec(lhs_q, wq_v, s_wq).astype(bf16)

    picked = {}
    for step, offsets in s_wuk:
        stream.wait(*step)
        for o in offsets:
            s = lax.dot_general(q, wuk_v[pl.ds(o, _HEAD_ROWS), :], _NT, preferred_element_type=f32)
            picked[o] = jnp.where(own_head[:, :_HEAD_ROWS], s * (D ** -0.5), 0.0).astype(bf16)
    picked = [jnp.concatenate([picked[o] for o in range(g, g + G, _HEAD_ROWS)], axis=1)
              for g in range(0, C * H, G)]
    qa = jnp.dot(jnp.concatenate(picked, axis=0), e_v[...], preferred_element_type=f32)
    qa = jnp.concatenate([qa[g * H:(g + 1) * H] for g in range(C // _LANES)], axis=1).astype(bf16)

    m = l = acc = None
    for step, offsets in s_kv:
        stream.wait(*step)
        c = jnp.concatenate([ckv_v[pl.ds(o, _KV_ROWS), :] for o in offsets], axis=0)
        s = lax.dot_general(qa, c, _NT, preferred_element_type=f32)
        m_blk = jnp.max(s, axis=-1, keepdims=True)
        m_new = m_blk if m is None else jnp.maximum(m, m_blk)
        p = jnp.exp(s - m_new)
        l_blk = jnp.sum(p, axis=-1, keepdims=True)
        pv = jnp.dot(p.astype(bf16), c, preferred_element_type=f32)
        if m is None:
            l, acc = l_blk, pv
        else:
            alpha = jnp.exp(m - m_new)
            l, acc = alpha * l + l_blk, alpha * acc + pv
        m = m_new
    lhs_v = spread(acc / l)

    ctx = per_head_matvec(lhs_v, wuv_v, s_wuv)

    sub = lax.broadcasted_iota(jnp.int32, (8, D), 0)
    lhs_o = jnp.concatenate(
        [jnp.where(sub == h % 8, ctx[h // 8 * 8:h // 8 * 8 + 8], 0.0) for h in range(H)],
        axis=1).astype(bf16)
    attn = None
    for step, offsets in s_wo:
        stream.wait(*step)
        for o in offsets:
            t = jnp.dot(lhs_o[:, o:o + _OUT_ROWS], wo_v[pl.ds(o, _OUT_ROWS), :],
                        preferred_element_type=f32)
            attn = t if attn is None else attn + t
    attn = jnp.sum(attn, axis=0, keepdims=True)
    h1 = x + attn
    hn = _layernorm(h1)

    hb = jnp.broadcast_to(hn, (_LANES, M)).astype(bf16)
    wr = wr_v[...].astype(f32)
    r = sum(jnp.sum(hn[:, i * _LANES:(i + 1) * _LANES] * wr[i:i + 1], axis=-1, keepdims=True)
            for i in range(M // _LANES))
    route = _sigmoid(r)
    act = []
    for bg, bu, (o, n) in zip(b_gate, b_up, ffn_rows):
        stream.wait(bg, bu)
        wg, wu = wg_v[pl.ds(o, n), :], wu_v[pl.ds(o, n), :]
        if act:
            gt = lax.dot_general(hb[:8], wg, _NT, preferred_element_type=f32)
            up = lax.dot_general(hb[:8], wu, _NT, preferred_element_type=f32)
        else:
            gt = lax.dot_general(wg, hb, _NT, preferred_element_type=f32)
            up = lax.dot_general(wu, hb, _NT, preferred_element_type=f32)
        act.append(gt * _sigmoid(gt) * up * route)
    act_col = act[0]
    act = jnp.concatenate(act[1:], axis=1).astype(bf16)

    first = lax.broadcasted_iota(jnp.int32, (8, M), 0) == 0
    y_v[...] = jnp.where(first, h1 + (hn + hn * 0.0), 0.0)
    for b, (o, n) in zip(b_early + b_down, [(0, _DOWN_EARLY)] + down_rows):
        stream.wait(b)
        w = wd_v[pl.ds(o, n), :]
        if o < vpu_rows[0]:
            t = jnp.where(first, jnp.dot(act[:, o:o + n], w, preferred_element_type=f32), 0.0)
        else:
            a = act_col[o - vpu_rows[0]:o - vpu_rows[0] + n]
            t = w.astype(f32) * jnp.concatenate([a] * (M // _LANES), axis=1)
            t = jnp.sum(t.reshape(n // 8, 8, M), axis=0)
        if o + n < F and _PIN:
            y_v[...] += t
        elif _PIN:
            o_ref[0] = jnp.sum(y_v[...] + t, axis=0, keepdims=True).astype(o_ref.dtype)
        else:
            y = (y_v[...] if o == 0 else y) + t
    if not _PIN:
        o_ref[0] = jnp.sum(y, axis=0, keepdims=True).astype(o_ref.dtype)


@jax.jit
def pallas_sequential_preLN__compressed_kv_cla__moe_arch_mod__decode_kernel(
    A_x: jax.Array,
    A_c_kv: jax.Array,
    A_w_q: jax.Array,
    A_w_uk: jax.Array,
    A_w_uv: jax.Array,
    A_w_o: jax.Array,
    B_x: jax.Array,
    B_w_r: jax.Array,
    B_w_gate: jax.Array,
    B_w_up: jax.Array,
    B_w_down: jax.Array,
):
    del B_x
    B, Sq, M = A_x.shape
    _, Sk, C = A_c_kv.shape
    _, H, D = A_w_q.shape
    F = B_w_gate.shape[1]
    assert B == 1 and Sq == 1 and D == _LANES
    assert M == C and sum(_FFN_CHUNKS) + sum(_DOWN_VPU) == F
    assert _DOWN_EARLY + sum(_DOWN_MXU) == sum(_FFN_CHUNKS)
    bf16 = jnp.bfloat16

    operands = (
        A_x,
        A_c_kv.reshape(Sk, C),
        A_w_q.reshape(M * H, D),
        A_w_uk.reshape(C * H, D),
        A_w_uv.reshape(C * H, D),
        A_w_o.reshape(H * D, M),
        B_w_r.reshape(M // _LANES, _LANES),
        B_w_gate.T,
        B_w_up.T,
        B_w_down,
    )
    n_copies = (2 + (M + 2 * C) * H // _HEAD_ROWS + Sk // _KV_ROWS + H * D // _OUT_ROWS
                + 2 * (1 + len(_FFN_CHUNKS)) + 1 + len(_DOWN_MXU) + len(_DOWN_VPU))

    def body(*refs):
        pl.run_scoped(lambda sems: _kernel(*refs, sems, heads=H, head_dim=D),
                      pltpu.SemaphoreType.DMA((n_copies,)))

    return pl.pallas_call(
        body,
        in_specs=[pl.BlockSpec(memory_space=pltpu.HBM)] * len(operands),
        out_specs=pl.BlockSpec(memory_space=pltpu.VMEM),
        out_shape=jax.ShapeDtypeStruct((B, Sq, M), A_x.dtype),
        scratch_shapes=[pltpu.VMEM(a.shape, a.dtype) for a in operands] + [
            pltpu.VMEM((_LANES * H, _LANES), bf16),
            pltpu.VMEM((8, M), jnp.float32)],
        compiler_params=pltpu.CompilerParams(vmem_limit_bytes=96 * 1024 * 1024),
    )(*operands)
```

```python
import jax
import jax.numpy as jnp
from jax import lax
import jax.experimental.pallas as pl
import jax.experimental.pallas.tpu as pltpu

_EPS = 1e-5
_LANES = 128
_NT = (((1,), (1,)), ((), ()))

_HEAD_ROWS = 512
_KV_ROWS = 256
_OUT_ROWS = 128
_FFN_ROWS = 128
_DOWN_EARLY = 640
_DOWN_MXU = (256, 256)
_DOWN_VPU = (128, 48, 32, 16)

_PIECE_BYTES = 32 * 1024
_LOOKAHEAD = 96
_START_STEPS = 4
_START_BYTES = 8 * 1024
_START_ISSUE = (210, 225)

_X, _CKV, _WQ, _WUK, _WUV, _WO, _WR, _WG, _WU, _WD = range(10)


def _consecutive(start, sizes):
    out = []
    for n in sizes:
        out.append((start, n))
        start += n
    return out


class _Plan:
    def __init__(self, operands):
        self._row_bytes = [a.shape[-1] * a.dtype.itemsize for a in operands]
        self._rows = [a.shape[0] for a in operands]
        self.blocks = []
        self.pieces = []
        self.ends = {}

        self.small = sum(self._add([(_X, 0, self._rows[_X])], [(_WR, 0, self._rows[_WR])]), [])
        self.wq = self._halves(_WQ, _HEAD_ROWS, _START_STEPS)
        self.wuk = self._halves(_WUK, _HEAD_ROWS)
        self.ckv = self._halves(_CKV, _KV_ROWS)
        self.wuv = self._halves(_WUV, _HEAD_ROWS)
        self.wo = self._halves(_WO, _OUT_ROWS)
        self.mxu_rows = _DOWN_EARLY + sum(_DOWN_MXU)
        assert self.mxu_rows % _FFN_ROWS == 0
        assert self.mxu_rows + sum(_DOWN_VPU) == self._rows[_WD]
        ffn = [(self.mxu_rows, sum(_DOWN_VPU))]
        ffn += _consecutive(0, (_FFN_ROWS,) * (self.mxu_rows // _FFN_ROWS))
        self.ffn = list(zip(*self._add([(_WG, *r) for r in ffn], [(_WU, *r) for r in ffn])))
        late, early = self._add(
            [(_WD, *r) for r in _consecutive(_DOWN_EARLY, _DOWN_MXU + _DOWN_VPU)],
            [(_WD, 0, _DOWN_EARLY)])
        self.down = early + late

    def _add(self, slow, fast, piece_bytes=_PIECE_BYTES):
        lanes, ids = [], []
        for queue, blocks in ((1, slow), (0, fast)):
            lanes.append([])
            ids.append([])
            for op, lo, n in blocks:
                step = piece_bytes // self._row_bytes[op]
                lanes[-1] += [(op, o, min(step, lo + n - o), len(self.blocks), queue)
                              for o in range(lo, lo + n, step)]
                ids[-1].append(len(self.blocks))
                self.blocks.append((op, lo, n))
        for i in range(max(len(lane) for lane in lanes)):
            for lane in lanes:
                if i < len(lane):
                    self.pieces.append(lane[i])
                    self.ends[lane[i][3]] = len(self.pieces)
        return ids

    def _halves(self, op, rows, small=0):
        half = self._rows[op] // 2
        assert half % rows == 0
        starts = range(0, half, rows)
        pairs = []
        for part, size in ((starts[:small], _START_BYTES), (starts[small:], _PIECE_BYTES)):
            pairs += zip(*self._add([(op, o, rows) for o in part],
                                    [(op, half + o, rows) for o in part], size))
        return pairs


class _Stream:
    def __init__(self, plan, src, dst, sems):
        self._plan, self._src, self._dst, self._sems = plan, src, dst, sems
        self._issued = 0
        self.pending = set(range(len(plan.blocks)))

    def issue(self, upto):
        for op, lo, n, block, queue in self._plan.pieces[self._issued:upto]:
            rows = pl.ds(lo, n)
            pltpu.make_async_copy(self._src[op].at[rows], self._dst[op].at[rows],
                                  self._sems.at[block]).start(priority=queue)
        self._issued = max(self._issued, upto)

    def take(self, *blocks):
        self.issue(max(self._plan.ends[b] for b in blocks) + _LOOKAHEAD)
        views = []
        for b in blocks:
            self.pending.remove(b)
            op, lo, n = self._plan.blocks[b]
            view = self._dst[op].at[pl.ds(lo, n)]
            pltpu.make_async_copy(view, view, self._sems.at[b]).wait()
            views.append((lo, view))
        return [(lo, view[...]) for lo, view in views]


def _layernorm(x):
    m = jnp.mean(x, axis=-1, keepdims=True)
    d = x - m
    v = jnp.mean(d * d, axis=-1, keepdims=True)
    return d / jnp.sqrt(v + _EPS)


def _sigmoid(x):
    return 1.0 / (1.0 + jnp.exp(-x))


def _dot(a, b):
    return jnp.dot(a, b, preferred_element_type=jnp.float32)


def _dot_nt(a, b):
    return lax.dot_general(a, b, _NT, preferred_element_type=jnp.float32)


def _compute(plan, stream, o_ref, e_ref, y_ref, H, D):
    f32, bf16 = jnp.float32, jnp.bfloat16
    M = o_ref.shape[-1]
    G = _LANES * H

    stream.issue(_START_ISSUE[0])
    e_ref[...] = jnp.where(lax.broadcasted_iota(jnp.int32, (G, _LANES), 0) // H
                           == lax.broadcasted_iota(jnp.int32, (G, _LANES), 1),
                           1.0, 0.0).astype(bf16)
    own_head = (lax.broadcasted_iota(jnp.int32, (H, G), 1) % H
                == lax.broadcasted_iota(jnp.int32, (H, G), 0))
    stream.issue(_START_ISSUE[1])

    def per_head_matvec(coef, steps):
        n = coef.shape[1] // _LANES
        stacked = jnp.concatenate(
            [coef[:, g * _LANES:(g + 1) * _LANES] for g in range(n)], axis=0).astype(bf16)
        rep = _dot_nt(stacked, e_ref[...])
        lhs = [jnp.where(own_head, rep[g * H:(g + 1) * H], 0.0).astype(bf16) for g in range(n)]
        acc = jnp.zeros((H, D), f32)
        for step in steps:
            for lo, w in stream.take(*step):
                acc += _dot(lhs[lo // G][:, lo % G:lo % G + w.shape[0]], w)
        return acc

    (_, x), (_, w_r) = stream.take(*plan.small)
    x = x[0].astype(f32)
    q = per_head_matvec(jnp.broadcast_to(_layernorm(x), (H, M)), plan.wq).astype(bf16)

    picked = {}
    for step in plan.wuk:
        for lo, w in stream.take(*step):
            s = _dot_nt(q, w) * (D ** -0.5)
            picked[lo] = jnp.where(own_head[:, :w.shape[0]], s, 0.0).astype(bf16)
    groups = len(picked) * _HEAD_ROWS // G
    picked = jnp.concatenate(
        [jnp.concatenate([picked[lo] for lo in range(g * G, (g + 1) * G, _HEAD_ROWS)], axis=1)
         for g in range(groups)], axis=0)
    qa = _dot(picked, e_ref[...])
    qa = jnp.concatenate([qa[g * H:(g + 1) * H] for g in range(groups)], axis=1).astype(bf16)

    m = None
    for step in plan.ckv:
        c = jnp.concatenate([w for _, w in stream.take(*step)], axis=0)
        s = _dot_nt(qa, c)
        m_new = jnp.max(s, axis=-1, keepdims=True)
        if m is not None:
            m_new = jnp.maximum(m, m_new)
        p = jnp.exp(s - m_new)
        p_sum = jnp.sum(p, axis=-1, keepdims=True)
        pc = _dot(p.astype(bf16), c)
        if m is None:
            l, acc = p_sum, pc
        else:
            alpha = jnp.exp(m - m_new)
            l, acc = alpha * l + p_sum, alpha * acc + pc
        m = m_new

    ctx = per_head_matvec(acc / l, plan.wuv)
    sub = lax.broadcasted_iota(jnp.int32, (8, D), 0)
    lhs_o = jnp.concatenate(
        [jnp.where(sub == h % 8, ctx[h // 8 * 8:h // 8 * 8 + 8], 0.0) for h in range(H)],
        axis=1).astype(bf16)
    attn = jnp.zeros((8, M), f32)
    for step in plan.wo:
        for lo, w in stream.take(*step):
            attn += _dot(lhs_o[:, lo:lo + w.shape[0]], w)
    h1 = x + jnp.sum(attn, axis=0, keepdims=True)
    hn = _layernorm(h1)

    w_r = w_r.astype(f32)
    r = sum(jnp.sum(hn[:, i * _LANES:(i + 1) * _LANES] * w_r[i:i + 1], axis=-1, keepdims=True)
            for i in range(M // _LANES))
    route = _sigmoid(r)
    hb = jnp.broadcast_to(hn, (_LANES, M)).astype(bf16)
    act = []
    for step in plan.ffn:
        (lo, w_gate), (_, w_up) = stream.take(*step)
        if lo < plan.mxu_rows:
            gate, up = _dot_nt(hb[:8], w_gate), _dot_nt(hb[:8], w_up)
            act.append((gate * _sigmoid(gate) * up * route).astype(bf16))
        else:
            gate, up = _dot_nt(w_gate, hb), _dot_nt(w_up, hb)
            act_col = gate * _sigmoid(gate) * up * route
    act = jnp.concatenate(act, axis=1)

    first = lax.broadcasted_iota(jnp.int32, (8, M), 0) == 0
    y_ref[...] = jnp.where(first, h1 + (hn + hn * 0.0), 0.0)
    for block in plan.down:
        (lo, w), = stream.take(block)
        n = w.shape[0]
        if lo < plan.mxu_rows:
            t = jnp.where(first, _dot(act[:, lo:lo + n], w), 0.0)
        else:
            a = act_col[lo - plan.mxu_rows:lo - plan.mxu_rows + n]
            t = w.astype(f32) * jnp.concatenate([a] * (M // _LANES), axis=1)
            t = jnp.sum(t.reshape(n // 8, 8, M), axis=0)
        if stream.pending:
            y_ref[...] += t
        else:
            o_ref[0] = jnp.sum(y_ref[...] + t, axis=0, keepdims=True).astype(o_ref.dtype)
    assert not stream.pending


@jax.jit
def pallas_sequential_preLN__compressed_kv_cla__moe_arch_mod__decode_kernel(
    A_x: jax.Array,
    A_c_kv: jax.Array,
    A_w_q: jax.Array,
    A_w_uk: jax.Array,
    A_w_uv: jax.Array,
    A_w_o: jax.Array,
    B_x: jax.Array,
    B_w_r: jax.Array,
    B_w_gate: jax.Array,
    B_w_up: jax.Array,
    B_w_down: jax.Array,
):
    del B_x
    B, Sq, M = A_x.shape
    _, Sk, C = A_c_kv.shape
    _, H, D = A_w_q.shape
    assert B == 1 and Sq == 1 and D == _LANES and M % _LANES == 0 and C % _LANES == 0

    operands = (
        A_x,
        A_c_kv.reshape(Sk, C),
        A_w_q.reshape(M * H, D),
        A_w_uk.reshape(C * H, D),
        A_w_uv.reshape(C * H, D),
        A_w_o.reshape(H * D, M),
        B_w_r.reshape(M // _LANES, _LANES),
        B_w_gate.T,
        B_w_up.T,
        B_w_down,
    )
    n = len(operands)
    plan = _Plan(operands)

    def kernel(*refs):
        src, o_ref, dst, (e_ref, y_ref) = refs[:n], refs[n], refs[n + 1:2 * n + 1], refs[2 * n + 1:]
        pl.run_scoped(
            lambda sems: _compute(plan, _Stream(plan, src, dst, sems), o_ref, e_ref, y_ref, H, D),
            pltpu.SemaphoreType.DMA((len(plan.blocks),)))

    return pl.pallas_call(
        kernel,
        in_specs=[pl.BlockSpec(memory_space=pltpu.HBM)] * n,
        out_specs=pl.BlockSpec(memory_space=pltpu.VMEM),
        out_shape=jax.ShapeDtypeStruct((B, Sq, M), A_x.dtype),
        scratch_shapes=[pltpu.VMEM(a.shape, a.dtype) for a in operands] + [
            pltpu.VMEM((_LANES * H, _LANES), jnp.bfloat16),
            pltpu.VMEM((8, M), jnp.float32),
        ],
        compiler_params=pltpu.CompilerParams(vmem_limit_bytes=64 * 1024 * 1024),
    )(*operands)
```
